```python
import os as _os
_os.environ.setdefault("JAX_PLATFORMS", "cpu")
import jax
import jax.numpy as jnp

def _softmax(x, axis=-1):
    return jax.nn.softmax(x, axis=axis)
def _gelu(x):
    return jax.nn.gelu(x, approximate=True)
def _silu(x):
    return jax.nn.silu(x)
def _sigmoid(x):
    return jax.nn.sigmoid(x)
def _layernorm(x, axis=-1, eps=1e-5):
    m = jnp.mean(x, axis=axis, keepdims=True)
    v = jnp.var(x, axis=axis, keepdims=True)
    return (x - m) / jnp.sqrt(v + eps)
def _scatter_add(tgt, idx, src, axis=0):
    return tgt.at[idx].add(src)
def _segment_sum(src, seg, n):
    return jax.ops.segment_sum(src, seg, n)
class _Rng:
    def __init__(self, key):
        self._k = key
    def _next(self):
        self._k, sub = jax.random.split(self._k)
        return sub
    def normal(self, shape):
        return jax.random.normal(self._next(), shape, dtype=jnp.bfloat16)
    def randint(self, lo, hi, shape):
        return jax.random.randint(self._next(), shape, lo, hi, dtype=jnp.int32)
    def uniform(self, shape, lo=0.0, hi=1.0):
        return jax.random.uniform(self._next(), shape, jnp.bfloat16, lo, hi)
    def permutation(self, n):
        return jax.random.permutation(self._next(), n)


kernel_name = 'standalone__mha_softmax__near_ridge'

def setup_inputs():
    _rng = _Rng(jax.random.key(int.from_bytes(__import__("os").urandom(4), "little")))
    _w = (lambda a: (lambda t: t.astype(jnp.bfloat16) if jnp.issubdtype(t.dtype, jnp.floating) else t)(jnp.asarray(a)))
    B, H, Sq, Sk, D = 8, 32, 304, 2048, 128
    return {
        "q": _w((lambda *s: _rng.normal(s) * 0.4)(B, H, Sq, D)),
        "k": _w((lambda *s: _rng.normal(s) * 0.4)(B, H, Sk, D)),
        "v": _w((lambda *s: _rng.normal(s) * 0.05)(B, H, Sk, D)),
    }

def reference(q, k, v):
    scale = q.shape[-1] ** -0.5
    scores = jnp.einsum("bhqd,bhkd->bhqk", q, k) * scale
    p = _softmax(scores, axis=-1)
    return jnp.einsum("bhqk,bhkd->bhqd", p, v)
```

```python
import math

import jax
import jax.numpy as jnp
from jax import lax
import jax.experimental.pallas as pl
import jax.experimental.pallas.tpu as pltpu

_NT = (((1,), (1,)), ((), ()))
_LOG2E = math.log2(math.e)

_HEADS_PER_STEP = 8


def _mha_kernel(q_ref, k_ref, v_ref, o_ref, *, heads_per_step):
    d = q_ref.shape[-1]
    c = (d ** -0.5) * _LOG2E
    for h in range(heads_per_step):
        q = q_ref[0, h]
        k = k_ref[0, h]
        v = v_ref[0, h]
        s = lax.dot_general(q, k, _NT,
                            preferred_element_type=jnp.float32)
        m = jnp.max(s, axis=-1, keepdims=True)
        p = jnp.exp2((s - m) * c)
        l = jnp.sum(p, axis=-1, keepdims=True)
        acc = jnp.dot(p.astype(jnp.bfloat16), v,
                      preferred_element_type=jnp.float32)
        r = pl.reciprocal(l, approx=True)
        r = r * (2.0 - l * r)
        o_ref[0, h] = (acc * r).astype(o_ref.dtype)


@jax.jit
def pallas_standalone__mha_softmax__near_ridge_kernel(
    q: jax.Array,
    k: jax.Array,
    v: jax.Array,
):
    b, h, sq, d = q.shape
    sk = k.shape[2]
    n = b * h
    hb = _HEADS_PER_STEP
    while n % hb:
        hb //= 2
    g = n // hb
    q4 = q.reshape(g, hb, sq, d)
    k4 = k.reshape(g, hb, sk, d)
    v4 = v.reshape(g, hb, sk, d)

    def idx(i):
        return (i, 0, 0, 0)

    kernel = lambda q_ref, k_ref, v_ref, o_ref: _mha_kernel(
        q_ref, k_ref, v_ref, o_ref, heads_per_step=hb)

    out = pl.pallas_call(
        kernel,
        grid=(g,),
        in_specs=[
            pl.BlockSpec((1, hb, sq, d), idx),
            pl.BlockSpec((1, hb, sk, d), idx),
            pl.BlockSpec((1, hb, sk, d), idx),
        ],
        out_specs=pl.BlockSpec((1, hb, sq, d), idx),
        out_shape=jax.ShapeDtypeStruct((g, hb, sq, d), q.dtype),
        compiler_params=pltpu.CompilerParams(
            dimension_semantics=("arbitrary",),
            vmem_limit_bytes=96 * 1024 * 1024,
        ),
    )(q4, k4, v4)
    return out.reshape(b, h, sq, d)
```

```python
import math

import jax
import jax.numpy as jnp
from jax import lax
import jax.experimental.pallas as pl
import jax.experimental.pallas.tpu as pltpu

_NT = (((1,), (1,)), ((), ()))
_LOG2E = math.log2(math.e)

_HEADS_PER_STEP = 8
_KEY_CHUNKS = 4


def _lane_fold(x, op):
    r = x[:, :128]
    for t in range(1, x.shape[1] // 128):
        r = op(r, x[:, t * 128:(t + 1) * 128])
    return r


def _mha_kernel(q_ref, k_ref, v_ref, o_ref, *, heads_per_step, key_chunks):
    d = q_ref.shape[-1]
    sk = k_ref.shape[2]
    tk = sk // key_chunks
    c = (d ** -0.5) * _LOG2E
    for h in range(heads_per_step):
        q = q_ref[0, h]
        m = lsum = acc = None
        for j in range(key_chunks):
            sl = pl.ds(j * tk, tk)
            s = lax.dot_general(q, k_ref[0, h, sl, :], _NT,
                                preferred_element_type=jnp.float32)
            mj = jnp.max(s, axis=-1, keepdims=True)
            if m is None:
                m_new = mj
            else:
                m_new = jnp.maximum(m, mj)
                alpha = jnp.exp2((m - m_new) * c)
                lsum = lsum * alpha
                acc = acc * alpha
            p = jnp.exp2((s - m_new) * c)
            lf = _lane_fold(p, jnp.add)
            lsum = lf if lsum is None else lsum + lf
            pv = jnp.dot(p.astype(jnp.bfloat16), v_ref[0, h, sl, :],
                         preferred_element_type=jnp.float32)
            acc = pv if acc is None else acc + pv
            m = m_new
        l = jnp.sum(lsum, axis=-1, keepdims=True)
        r = pl.reciprocal(l, approx=True)
        r = r * (2.0 - l * r)
        o_ref[0, h] = (acc * r).astype(o_ref.dtype)


@jax.jit
def pallas_standalone__mha_softmax__near_ridge_kernel(
    q: jax.Array,
    k: jax.Array,
    v: jax.Array,
):
    b, h, sq, d = q.shape
    sk = k.shape[2]
    n = b * h
    hb = _HEADS_PER_STEP
    while n % hb:
        hb //= 2
    nc = _KEY_CHUNKS
    while nc > 1 and (sk % (nc * 128)):
        nc //= 2
    g = n // hb
    q4 = q.reshape(g, hb, sq, d)
    k4 = k.reshape(g, hb, sk, d)
    v4 = v.reshape(g, hb, sk, d)

    def idx(i):
        return (i, 0, 0, 0)

    kernel = lambda q_ref, k_ref, v_ref, o_ref: _mha_kernel(
        q_ref, k_ref, v_ref, o_ref, heads_per_step=hb, key_chunks=nc)

    out = pl.pallas_call(
        kernel,
        grid=(g,),
        in_specs=[
            pl.BlockSpec((1, hb, sq, d), idx),
            pl.BlockSpec((1, hb, sk, d), idx),
            pl.BlockSpec((1, hb, sk, d), idx),
        ],
        out_specs=pl.BlockSpec((1, hb, sq, d), idx),
        out_shape=jax.ShapeDtypeStruct((g, hb, sq, d), q.dtype),
        compiler_params=pltpu.CompilerParams(
            dimension_semantics=("arbitrary",),
            vmem_limit_bytes=96 * 1024 * 1024,
        ),
    )(q4, k4, v4)
    return out.reshape(b, h, sq, d)
```
